```python
import os as _os
_os.environ.setdefault("JAX_PLATFORMS", "cpu")
import jax
import jax.numpy as jnp

def _softmax(x, axis=-1):
    return jax.nn.softmax(x, axis=axis)
def _gelu(x):
    return jax.nn.gelu(x, approximate=True)
def _silu(x):
    return jax.nn.silu(x)
def _sigmoid(x):
    return jax.nn.sigmoid(x)
def _layernorm(x, axis=-1, eps=1e-5):
    m = jnp.mean(x, axis=axis, keepdims=True)
    v = jnp.var(x, axis=axis, keepdims=True)
    return (x - m) / jnp.sqrt(v + eps)
def _scatter_add(tgt, idx, src, axis=0):
    return tgt.at[idx].add(src)
def _segment_sum(src, seg, n):
    return jax.ops.segment_sum(src, seg, n)
class _Rng:
    def __init__(self, key):
        self._k = key
    def _next(self):
        self._k, sub = jax.random.split(self._k)
        return sub
    def normal(self, shape):
        return jax.random.normal(self._next(), shape, dtype=jnp.bfloat16)
    def randint(self, lo, hi, shape):
        return jax.random.randint(self._next(), shape, lo, hi, dtype=jnp.int32)
    def uniform(self, shape, lo=0.0, hi=1.0):
        return jax.random.uniform(self._next(), shape, jnp.bfloat16, lo, hi)
    def permutation(self, n):
        return jax.random.permutation(self._next(), n)


kernel_name = 'concat_heads__sliding_local_dilated__compressed_kv_cla__prompt'

def setup_inputs():
    _rng = _Rng(jax.random.key(int.from_bytes(__import__("os").urandom(4), "little")))
    _w = (lambda a: (lambda t: t.astype(jnp.bfloat16) if jnp.issubdtype(t.dtype, jnp.floating) else t)(jnp.asarray(a)))
    def _A_setup():
        B, S, D = 1, 2048, 640
        return {
            "x": _w((lambda *s: _rng.normal(s) * 0.2)(B, S, D)),
            "wqkv": _w((lambda *s: _rng.normal(s) * 0.2)(D, 3 * D)),
            "wo": _w((lambda *s: _rng.normal(s) * 0.05)(D, D)),
        }
    _A_in = _A_setup()

    def _B_setup():
        B, H, Sq, Sk, D, M = 1, 32, 2048, 2048, 128, 640
        Dc = 4 * D
        return {
            "x": _w((lambda *s: _rng.normal(s) * 0.8)(B, Sq, M)),
            "c_kv": _w((lambda *s: _rng.normal(s) * 0.8)(B, Sk, Dc)),
            "w_q": _w((lambda *s: _rng.normal(s) * 1.6)(M, H, D) * (M ** -0.5)),
            "w_uk": _w((lambda *s: _rng.normal(s) * 1.6)(Dc, H, D) * (Dc ** -0.5)),
            "w_uv": _w((lambda *s: _rng.normal(s) * 0.8)(Dc, H, D) * (Dc ** -0.5)),
            "w_o": _w((lambda *s: _rng.normal(s) * 0.8)(H, D, M) * ((H * D) ** -0.5)),
        }
    _B_in = _B_setup()

    return {
        "A_x": _A_in["x"],
        "A_wqkv": _A_in["wqkv"],
        "A_wo": _A_in["wo"],
        "B_x": _B_in["x"],
        "B_c_kv": _B_in["c_kv"],
        "B_w_q": _B_in["w_q"],
        "B_w_uk": _B_in["w_uk"],
        "B_w_uv": _B_in["w_uv"],
        "B_w_o": _B_in["w_o"],
    }

def reference(A_x, A_wqkv, A_wo, B_x, B_c_kv, B_w_q, B_w_uk, B_w_uv, B_w_o):
    def _A_ref(x, wqkv, wo):
        B, S, D = x.shape
        H = 32; Dh = D // H
        W, dil = 8, 2
        qkv = (lambda x, *d: x.transpose(*d))((x @ wqkv).reshape(B, S, 3, H, Dh), 2, 0, 3, 1, 4)
        q, k, v = qkv[0], qkv[1], qkv[2]
        scale = Dh ** -0.5
        pos = jnp.arange(S)
        off = jnp.arange(W) * dil
        idx = pos[:, None] - off[None, :]
        mask = idx >= 0
        idx_c = jnp.where(mask, idx, 0).reshape(-1)
        kg = k[:, :, idx_c, :].reshape(B, H, S, W, Dh)
        vg = v[:, :, idx_c, :].reshape(B, H, S, W, Dh)
        logits = jnp.einsum("bhsd,bhswd->bhsw", q, kg) * scale
        logits = jnp.where(mask[None, None, :, :], logits, -1e9)
        attn = _softmax(logits, axis=-1)
        o = jnp.einsum("bhsw,bhswd->bhsd", attn, vg)
        return (lambda x, *d: x.transpose(*d))(o, 0, 2, 1, 3).reshape(B, S, D) @ wo

    def _B_ref(x, c_kv, w_q, w_uk, w_uv, w_o):
        B, Sq, M = x.shape[0], x.shape[1], x.shape[2]
        Sk = c_kv.shape[1]
        H, D = w_q.shape[1], w_q.shape[2]
        q = jnp.einsum("bqm,mhd->bhqd", x, w_q)
        k = jnp.einsum("bkc,chd->bhkd", c_kv, w_uk)
        v = jnp.einsum("bkc,chd->bhkd", c_kv, w_uv)
        scores = jnp.einsum("bhqd,bhkd->bhqk", q, k) * (D ** -0.5)
        off = Sk - Sq
        qi = jnp.arange(Sq)[:, None]
        kj = jnp.arange(Sk)[None, :]
        cmask = kj <= (qi + off)
        scores = jnp.where(cmask[None, None], scores, -1e9)
        p = _softmax(scores, axis=-1)
        ctx = jnp.einsum("bhqk,bhkd->bhqd", p, v)
        return jnp.einsum("bhqd,hdm->bqm", ctx, w_o)

    a = _A_ref(A_x, A_wqkv, A_wo)
    b = _B_ref(B_x, B_c_kv, B_w_q, B_w_uk, B_w_uv, B_w_o)
    return jnp.concatenate([a, b], axis=-1)
```

```python
import math

import jax
import jax.numpy as jnp
from jax import lax
import jax.experimental.pallas as pl
import jax.experimental.pallas.tpu as pltpu

F32 = jnp.float32
BF16 = jnp.bfloat16
LOG2E = math.log2(math.e)
NT = (((1,), (1,)), ((), ()))

A_HEADS = 32
A_WIN = 8
A_DIL = 2
HALO = 16
G = 4
BQ = 512
RC = 32
WR = 16
PR = 128
WQ, WK, WV, WO = (1, 2, 2, 1), (1, 1, 1, 1), (1, 1, 1, 0), (1, 1, 1, 0)
BLOCK_ORDER = (2, 3, 1, 0)
NO = 4
NCH = 4
T = 128


def _dot(a, b):
    return jnp.dot(a, b, preferred_element_type=F32)


def _dot_nt(a, b):
    return lax.dot_general(a, b, NT, preferred_element_type=F32)


def _pack(x):
    return pltpu.bitcast(x, jnp.uint32)


def _unpack(x):
    return pltpu.bitcast(x, BF16)


def _recip(x):
    r = pl.reciprocal(x, approx=True)
    return r * (2.0 - x * r)


def _rows(ref, h, lo, hi):
    return _unpack(ref[h, lo // 2:hi // 2, :])


def _causal_head(q_ref, k_ref, v_ref, ctx_ref, s_refs, p_refs, h, seq):
    nt = BQ // T
    col = lax.broadcasted_iota(jnp.int32, (RC, T), 1)
    row = lax.broadcasted_iota(jnp.int32, (RC, T), 0)

    def scores(r0, s_ref):
        for c in range(nt):
            hi = r0 + (c + 1) * T
            s_ref[c * T:(c + 1) * T, :hi] = _dot_nt(_rows(q_ref, h, hi - T, hi), _rows(k_ref, h, 0, hi))

    def softmax(r0, s_ref, p_ref):
        inv_l = []
        for a in range(0, BQ, RC):
            last = (r0 + a) // T

            def tile(j):
                x = s_ref[a:a + RC, j * T:(j + 1) * T]
                return jnp.where(col <= row + a % T, x, -1e9) if j == last else x

            m = tile(0)
            for j in range(1, last + 1):
                m = jnp.maximum(m, tile(j))
            m = jnp.max(m, axis=1, keepdims=True)
            l = None
            for j in range(last + 1):
                p_ref[a // 2:(a + RC) // 2, j * T:(j + 1) * T] = _pack(jnp.exp2(tile(j) - m).astype(BF16))
            for j in range(last + 1):
                e = _unpack(p_ref[a // 2:(a + RC) // 2, j * T:(j + 1) * T]).astype(F32)
                l = e if l is None else l + e
            inv_l.append(_recip(jnp.sum(l, axis=1, keepdims=True)))
        return inv_l

    def context(r0, p_ref, inv_l):
        for c in range(nt):
            hi = r0 + (c + 1) * T
            o = _dot(_unpack(p_ref[c * T // 2:(c + 1) * T // 2, :hi]), _rows(v_ref, h, 0, hi))
            for a in range(0, T, RC):
                lo = r0 + c * T + a
                ctx_ref[h, lo // 2:(lo + RC) // 2, :] = _pack(
                    (o[a:a + RC] * inv_l[(c * T + a) // RC]).astype(BF16))

    blocks = [BQ * b for b in BLOCK_ORDER]
    assert sorted(blocks) == list(range(0, seq, BQ))
    scores(blocks[0], s_refs[0])
    for i, r0 in enumerate(blocks):
        if i + 1 < len(blocks):
            scores(blocks[i + 1], s_refs[(i + 1) % 2])
        context(r0, p_refs[i % 2], softmax(r0, s_refs[i % 2], p_refs[i % 2]))


def _window_rows(qa_ref, ka_ref, va_ref, oa_ref, lo, pos0, rows):
    nv = qa_ref.shape[1] // 128
    q = [qa_ref[lo:lo + rows, j * 128:(j + 1) * 128] for j in range(nv)]
    pos = pos0 + lax.broadcasted_iota(jnp.int32, (rows, 128), 0)
    logits = []
    for w in range(A_WIN):
        a = HALO - w * A_DIL
        acc = q[0] * ka_ref[lo + a:lo + a + rows, 0:128]
        for j in range(1, nv):
            acc = acc + q[j] * ka_ref[lo + a:lo + a + rows, j * 128:(j + 1) * 128]
        acc = acc + pltpu.roll(acc, 64, 1)
        acc = acc + pltpu.roll(acc, 32, 1)
        logits.append(jnp.where(pos >= w * A_DIL, acc, -1e9) if w else acc)
    m = logits[0]
    for x in logits[1:]:
        m = jnp.maximum(m, x)
    ps = [jnp.exp2(x - m) for x in logits]
    l = ps[0]
    for x in ps[1:]:
        l = l + x
    inv = _recip(l)
    for j in range(nv):
        o = ps[0] * va_ref[lo + HALO:lo + HALO + rows, j * 128:(j + 1) * 128]
        for w in range(1, A_WIN):
            a = HALO - w * A_DIL
            o = o + ps[w] * va_ref[lo + a:lo + a + rows, j * 128:(j + 1) * 128]
        oa_ref[lo:lo + rows, j * 128:(j + 1) * 128] = (o * inv).astype(BF16)


def _split_heads(raw_ref, slot):
    cols = []
    for j in range(G // 2):
        w = raw_ref[slot, j]
        cols.append(pltpu.bitcast(w << 16, F32).astype(BF16))
        cols.append(pltpu.bitcast(w & jnp.uint32(0xFFFF0000), F32).astype(BF16))
    return jnp.concatenate(cols, axis=1)


def _kernel(ax_ref, wqkv_hbm, wo_hbm, bx_hbm, c_hbm, wq_hbm, wuk_hbm, wuv_hbm, wob_hbm,
            out_hbm,
            wa_raw, wa_p, wo_f32, wob_ref, bx_ref, c_ref, qa_ref, ka_ref, va_ref, oa_ref,
            q_ref, k_ref, v_ref, ctx_ref, acc_ref, wq_raw, wuk_raw, wuv_raw,
            s0, s1, p0, p1, outa_ref, outb_ref, sems, in_sems, out_sems):
    g = pl.program_id(0)
    last_step = pl.num_programs(0) - 1
    seq, dm = bx_ref.shape
    rows_a = ax_ref.shape[0]
    dh = dm // A_HEADS
    d = 128
    slot = g % 2
    a0 = pl.multiple_of(g * rows_a, rows_a)

    def weight_copies(step, slot):
        cps = []
        for i, (hbm, raw) in enumerate(((wq_hbm, wq_raw), (wuk_hbm, wuk_raw), (wuv_hbm, wuv_raw))):
            for j in range(G // 2):
                cps.append(pltpu.make_async_copy(
                    hbm.bitcast(jnp.uint32).at[:, step * (G // 2) + j, :],
                    raw.at[slot, j], sems.at[slot, i, j]))
        return cps

    def wa_copy(i):
        return pltpu.make_async_copy(
            wqkv_hbm.at[:, pl.ds(pl.multiple_of(i * dm, 128), dm)], wa_raw.at[i], in_sems.at[i])

    def out_a_copy(row0):
        return pltpu.make_async_copy(
            outa_ref, out_hbm.at[pl.ds(row0, rows_a), pl.ds(0, dm)], out_sems.at[NO])

    def out_b_copy(i):
        rs = pl.ds(i * (seq // NO), seq // NO)
        return pltpu.make_async_copy(outb_ref.at[rs], out_hbm.at[rs, pl.ds(dm, dm)], out_sems.at[i])

    x_cps = [pltpu.make_async_copy(bx_hbm, bx_ref, in_sems.at[4]),
             pltpu.make_async_copy(c_hbm, c_ref, in_sems.at[5])]

    wob_cp = pltpu.make_async_copy(wob_hbm.at[pl.ds(g * (G * d), G * d)], wob_ref, in_sems.at[6])
    wo_cp = pltpu.make_async_copy(wo_hbm, wa_raw.at[3], in_sems.at[3])

    @pl.when(g == 0)
    def _():
        w_cps = weight_copies(0, 0)
        stages = [[x_cps[0]] + w_cps[:G // 2], [], [x_cps[1]] + w_cps[G // 2:]]
        for i in range(3):
            wa_copy(i).start()
        ka_ref[rows_a:, :] = jnp.zeros((HALO, dm), F32)
        va_ref[rows_a:, :] = jnp.zeros((HALO, dm), F32)
        acc_ref[...] = jnp.zeros_like(acc_ref)
        lane = lax.broadcasted_iota(jnp.int32, (PR // 2, 128), 1)

        def permute(i, carry):
            wa_copy(i).wait()
            for n, stage in enumerate(stages):
                @pl.when(i == n)
                def _():
                    for cp in stage:
                        cp.start()

            def chunk(rr, carry):
                rs = pl.ds(pl.multiple_of(rr * PR, PR), PR)
                w = [_pack(wa_raw[i, rs, j * 128:(j + 1) * 128]) for j in range(dm // 128)]
                for j in range(dm // 128):
                    c = lane + j * 128
                    src = (c % A_HEADS) * dh + c // A_HEADS
                    o = w[0]
                    for jj in range(1, dm // 128):
                        o = jnp.where((lane + jj * 128) % dh // (128 // A_HEADS) == j, w[jj], o)
                    wa_p[i, rs, j * 128:(j + 1) * 128] = _unpack(
                        jnp.take_along_axis(o, src % 128, axis=1))
                return carry

            return lax.fori_loop(0, dm // PR, chunk, carry)

        lax.fori_loop(0, 3, permute, 0)

    @pl.when(g > 0)
    def _():
        out_a_copy(a0 - rows_a).wait()

    ax = ax_ref[...]
    qa_ref[...] = _dot(ax, wa_p[0]) * (dh ** -0.5 * LOG2E)
    ka_ref[:HALO, :] = ka_ref[rows_a:, :]
    va_ref[:HALO, :] = va_ref[rows_a:, :]
    ka_ref[HALO:, :] = _dot(ax, wa_p[1])
    va_ref[HALO:, :] = _dot(ax, wa_p[2])

    @pl.when(g == 0)
    def _():
        for cp in x_cps:
            cp.wait()
        wo_cp.start()

    wob_cp.start()

    for cp in weight_copies(g, slot):
        cp.wait()
    @pl.when(g < last_step)
    def _():
        for cp in weight_copies(g + 1, 1 - slot):
            cp.start()

    wq = _split_heads(wq_raw, slot)
    wk = _split_heads(wuk_raw, slot)
    wv = _split_heads(wuv_raw, slot)
    pieces = iter(range(0, rows_a, WR))

    def window_piece(n=1):
        for _ in range(n):
            lo = next(pieces)
            _window_rows(qa_ref, ka_ref, va_ref, oa_ref, lo, a0 + lo, WR)

    rc = seq // NCH
    for i in range(NCH):
        rs = slice(i * rc, (i + 1) * rc)
        qq = _dot(bx_ref[rs, :], wq) * (d ** -0.5 * LOG2E)
        window_piece(WQ[i])
        kk = _dot(c_ref[rs, :], wk)
        window_piece(WK[i])
        vv = _dot(c_ref[rs, :], wv)
        for h in range(G):
            hs = slice(i * rc // 2, (i + 1) * rc // 2)
            q_ref[h, hs, :] = _pack(qq[:, h * d:(h + 1) * d].astype(BF16))
            k_ref[h, hs, :] = _pack(kk[:, h * d:(h + 1) * d].astype(BF16))
            v_ref[h, hs, :] = _pack(vv[:, h * d:(h + 1) * d].astype(BF16))
        window_piece(WV[i])

    @pl.when(g == 0)
    def _():
        wo_cp.wait()

        def permute_rows(j, carry):
            cs = pl.ds(pl.multiple_of(j * 128, 128), 128)
            wo_f32[:dm, :] = wa_raw[3, :, cs].astype(F32)
            for i in range(dh):
                wa_p[3, i * A_HEADS:(i + 1) * A_HEADS, cs] = (
                    wo_f32[pl.ds(i, A_HEADS, stride=dh), :].astype(BF16))
            return carry

        lax.fori_loop(0, dm // 128, permute_rows, 0)

    wob_cp.wait()

    def body(h, carry):
        _causal_head(q_ref, k_ref, v_ref, ctx_ref, (s0, s1), (p0, p1), h, seq)
        return carry

    lax.fori_loop(0, G, body, 0)

    ro = seq // NO
    for i in range(NO):
        ctx = jnp.concatenate([_rows(ctx_ref, h, i * ro, (i + 1) * ro) for h in range(G)], axis=1)
        acc = acc_ref[i * ro:(i + 1) * ro, :] + _dot(ctx, wob_ref[...])
        acc_ref[i * ro:(i + 1) * ro, :] = acc
        outb_ref[i * ro:(i + 1) * ro, :] = acc.astype(BF16)
        window_piece(WO[i])
        if i == NO - 1:
            assert next(pieces, None) is None
            outa_ref[...] = _dot(oa_ref[...], wa_p[3]).astype(BF16)
            out_a_copy(a0).start()

        if i == NO - 2:
            @pl.when(g == last_step)
            def _():
                for n in range(NO - 1):
                    out_b_copy(n).start()

    @pl.when(g == last_step)
    def _():
        out_b_copy(NO - 1).start()
        out_a_copy(a0).wait()
        for i in range(NO):
            out_b_copy(i).wait()


@jax.jit
def pallas_concat_heads__sliding_local_dilated__compressed_kv_cla__prompt_kernel(
    A_x: jax.Array,
    A_wqkv: jax.Array,
    A_wo: jax.Array,
    B_x: jax.Array,
    B_c_kv: jax.Array,
    B_w_q: jax.Array,
    B_w_uk: jax.Array,
    B_w_uv: jax.Array,
    B_w_o: jax.Array,
):
    _, seq, dm = A_x.shape
    dc = B_c_kv.shape[-1]
    heads, d = B_w_q.shape[1:]
    steps = heads // G
    rows_a = seq // steps

    hbm = pl.BlockSpec(memory_space=pl.ANY)
    out = pl.pallas_call(
        _kernel,
        grid=(steps,),
        in_specs=[pl.BlockSpec((rows_a, dm), lambda g: (g, 0))] + [hbm] * 8,
        out_specs=hbm,
        out_shape=jax.ShapeDtypeStruct((seq, 2 * dm), BF16),
        scratch_shapes=[
            pltpu.VMEM((4, dm, dm), BF16),
            pltpu.VMEM((4, dm, dm), BF16),
            pltpu.VMEM((dm + A_HEADS, 128), F32),
            pltpu.VMEM((G * d, dm), BF16),
            pltpu.VMEM((seq, dm), BF16),
            pltpu.VMEM((seq, dc), BF16),
            pltpu.VMEM((rows_a, dm), F32),
            pltpu.VMEM((rows_a + HALO, dm), F32),
            pltpu.VMEM((rows_a + HALO, dm), F32),
            pltpu.VMEM((rows_a, dm), BF16),
            pltpu.VMEM((G, seq // 2, d), jnp.uint32),
            pltpu.VMEM((G, seq // 2, d), jnp.uint32),
            pltpu.VMEM((G, seq // 2, d), jnp.uint32),
            pltpu.VMEM((G, seq // 2, d), jnp.uint32),
            pltpu.VMEM((seq, dm), F32),
            pltpu.VMEM((2, G // 2, dm, d), jnp.uint32),
            pltpu.VMEM((2, G // 2, dc, d), jnp.uint32),
            pltpu.VMEM((2, G // 2, dc, d), jnp.uint32),
            pltpu.VMEM((BQ, seq), F32),
            pltpu.VMEM((BQ, seq), F32),
            pltpu.VMEM((BQ // 2, seq), jnp.uint32),
            pltpu.VMEM((BQ // 2, seq), jnp.uint32),
            pltpu.VMEM((rows_a, dm), BF16),
            pltpu.VMEM((seq, dm), BF16),
            pltpu.SemaphoreType.DMA((2, 3, G // 2)),
            pltpu.SemaphoreType.DMA((7,)),
            pltpu.SemaphoreType.DMA((NO + 1,)),
        ],
        compiler_params=pltpu.CompilerParams(
            dimension_semantics=("arbitrary",),
            vmem_limit_bytes=100 * 1024 * 1024,
        ),
    )(
        A_x.reshape(seq, dm), A_wqkv, A_wo,
        B_x.reshape(seq, dm), B_c_kv.reshape(seq, dc),
        B_w_q, B_w_uk, B_w_uv, B_w_o.reshape(heads * d, dm),
    )
    return out.reshape(1, seq, 2 * dm)
```
